```python
import os as _os
_os.environ.setdefault("JAX_PLATFORMS", "cpu")
import jax
import jax.numpy as jnp

def _softmax(x, axis=-1):
    return jax.nn.softmax(x, axis=axis)
def _gelu(x):
    return jax.nn.gelu(x, approximate=True)
def _silu(x):
    return jax.nn.silu(x)
def _sigmoid(x):
    return jax.nn.sigmoid(x)
def _layernorm(x, axis=-1, eps=1e-5):
    m = jnp.mean(x, axis=axis, keepdims=True)
    v = jnp.var(x, axis=axis, keepdims=True)
    return (x - m) / jnp.sqrt(v + eps)
def _scatter_add(tgt, idx, src, axis=0):
    return tgt.at[idx].add(src)
def _segment_sum(src, seg, n):
    return jax.ops.segment_sum(src, seg, n)
class _Rng:
    def __init__(self, key):
        self._k = key
    def _next(self):
        self._k, sub = jax.random.split(self._k)
        return sub
    def normal(self, shape):
        return jax.random.normal(self._next(), shape, dtype=jnp.bfloat16)
    def randint(self, lo, hi, shape):
        return jax.random.randint(self._next(), shape, lo, hi, dtype=jnp.int32)
    def uniform(self, shape, lo=0.0, hi=1.0):
        return jax.random.uniform(self._next(), shape, jnp.bfloat16, lo, hi)
    def permutation(self, n):
        return jax.random.permutation(self._next(), n)


kernel_name = 'standalone__gqa_block_cached__near_ridge'

def setup_inputs():
    _rng = _Rng(jax.random.key(int.from_bytes(__import__("os").urandom(4), "little")))
    _w = (lambda a: (lambda t: t.astype(jnp.bfloat16) if jnp.issubdtype(t.dtype, jnp.floating) else t)(jnp.asarray(a)))
    B, Sq, D = 8, 96, 640
    Hq, Hkv, Sk, Dh = 32, 32, 512, 128
    assert Hq % Hkv == 0, (Hq, Hkv)
    return {
        "x": _w((lambda *s: _rng.normal(s) * 0.2)(B, Sq, D)),
        "k_cache": _w((lambda *s: _rng.normal(s) * 3.2)(B, Hkv, Sk, Dh)),
        "v_cache": _w((lambda *s: _rng.normal(s) * 0.05)(B, Hkv, Sk, Dh)),
        "wq": _w((lambda *s: _rng.normal(s) * 0.2)(D, Hq * Dh) * (D ** -0.5)),
        "wo": _w((lambda *s: _rng.normal(s) * 0.05)(Hq * Dh, D) * ((Hq * Dh) ** -0.5)),
    }

def reference(x, k_cache, v_cache, wq, wo):
    B, Sq, D = x.shape
    Hq, Dh = 32, 128
    Hkv = k_cache.shape[1]
    rep = Hq // Hkv
    q = (lambda x, *d: x.transpose(*d))((x @ wq).reshape(B, Sq, Hq, Dh), 0, 2, 1, 3)
    k = jnp.repeat(k_cache, rep, axis=1)
    v = jnp.repeat(v_cache, rep, axis=1)
    scores = jnp.einsum("bhqd,bhkd->bhqk", q, k) * (Dh ** -0.5)
    p = _softmax(scores, axis=-1)
    o = jnp.einsum("bhqk,bhkd->bhqd", p, v)
    return (lambda x, *d: x.transpose(*d))(o, 0, 2, 1, 3).reshape(B, Sq, Hq * Dh) @ wo
```

```python
import jax
import jax.numpy as jnp
import jax.experimental.pallas as pl
import jax.experimental.pallas.tpu as pltpu

_G = 4
_BB = 2
_LOOK = 1
_LOG2E = 1.4426950408889634


@jax.jit
def pallas_standalone__gqa_block_cached__near_ridge_kernel(
    x: jax.Array,
    k_cache: jax.Array,
    v_cache: jax.Array,
    wq: jax.Array,
    wo: jax.Array,
):
    B, Sq, D = x.shape
    _, Hkv, Sk, Dh = k_cache.shape
    Hq = wq.shape[1] // Dh
    assert Hq == Hkv
    G, BB, LOOK = _G, _BB, _LOOK
    M = B * Sq
    c = (Dh ** -0.5) * _LOG2E
    nsteps = Hq // G
    x2 = x.reshape(M, D)

    def kernel(x_ref, k_hbm, v_hbm, wq_ref, wo_ref, o_ref,
               acc_ref, oall_ref, kbuf, vbuf, sems):
        step = pl.program_id(0)
        slot = step % 2

        def kcopy(st, sl, b):
            return pltpu.make_async_copy(
                k_hbm.at[b, pl.ds(st * G, G)], kbuf.at[sl, b], sems.at[0, sl, b])

        def vcopy(st, sl, b):
            return pltpu.make_async_copy(
                v_hbm.at[b, pl.ds(st * G, G)], vbuf.at[sl, b], sems.at[1, sl, b])

        @pl.when(step == 0)
        def _():
            for b in range(B):
                kcopy(0, 0, b).start()
                vcopy(0, 0, b).start()
            acc_ref[...] = jnp.zeros_like(acc_ref)

        @pl.when(step + 1 < nsteps)
        def _():
            for b in range(B):
                kcopy(step + 1, 1 - slot, b).start()
                vcopy(step + 1, 1 - slot, b).start()

        q_parts = []
        for bb in range(B // BB):
            rows = slice(bb * BB * Sq, (bb + 1) * BB * Sq)
            q_parts.append(
                jnp.dot(x_ref[rows, :], wq_ref[...],
                        preferred_element_type=jnp.float32).astype(jnp.bfloat16))

        items = [(b, g) for b in range(B) for g in range(G)]

        def qk(b, g):
            if g == 0:
                kcopy(step, slot, b).wait()
            qp = q_parts[b // BB]
            bi = b % BB
            q = qp[bi * Sq:(bi + 1) * Sq, g * Dh:(g + 1) * Dh]
            return jax.lax.dot_general(
                q, kbuf[slot, b, g], (((1,), (1,)), ((), ())),
                preferred_element_type=jnp.float32)

        pending = [qk(*it) for it in items[:LOOK]]
        for idx, (b, g) in enumerate(items):
            s = pending.pop(0)
            if idx + LOOK < len(items):
                pending.append(qk(*items[idx + LOOK]))
            m = jnp.max(s, axis=-1, keepdims=True)
            p = jnp.exp2((s - m) * c)
            l = jnp.sum(p, axis=-1, keepdims=True)
            if g == 0:
                vcopy(step, slot, b).wait()
            o = jnp.dot(p.astype(jnp.bfloat16), vbuf[slot, b, g],
                        preferred_element_type=jnp.float32)
            o = o / l
            oall_ref[b * Sq:(b + 1) * Sq, g * Dh:(g + 1) * Dh] = o.astype(jnp.bfloat16)
            if g == G - 1 and (b + 1) % BB == 0:
                rows = slice((b + 1 - BB) * Sq, (b + 1) * Sq)
                acc_ref[rows, :] += jnp.dot(
                    oall_ref[rows, :], wo_ref[...],
                    preferred_element_type=jnp.float32)

        @pl.when(step == nsteps - 1)
        def _():
            o_ref[...] = acc_ref[...].astype(o_ref.dtype)

    out = pl.pallas_call(
        kernel,
        grid=(nsteps,),
        in_specs=[
            pl.BlockSpec((M, D), lambda i: (0, 0)),
            pl.BlockSpec(memory_space=pl.ANY),
            pl.BlockSpec(memory_space=pl.ANY),
            pl.BlockSpec((D, G * Dh), lambda i: (0, i)),
            pl.BlockSpec((G * Dh, D), lambda i: (i, 0)),
        ],
        out_specs=pl.BlockSpec((M, D), lambda i: (0, 0)),
        out_shape=jax.ShapeDtypeStruct((M, D), x.dtype),
        scratch_shapes=[
            pltpu.VMEM((M, D), jnp.float32),
            pltpu.VMEM((M, G * Dh), jnp.bfloat16),
            pltpu.VMEM((2, B, G, Sk, Dh), jnp.bfloat16),
            pltpu.VMEM((2, B, G, Sk, Dh), jnp.bfloat16),
            pltpu.SemaphoreType.DMA((2, 2, B)),
        ],
        compiler_params=pltpu.CompilerParams(
            dimension_semantics=("arbitrary",),
            vmem_limit_bytes=100 * 1024 * 1024,
        ),
    )(x2, k_cache, v_cache, wq, wo)
    return out.reshape(B, Sq, D)
```
